```python
import os as _os
_os.environ.setdefault("JAX_PLATFORMS", "cpu")
import jax
import jax.numpy as jnp

def _softmax(x, axis=-1):
    return jax.nn.softmax(x, axis=axis)
def _gelu(x):
    return jax.nn.gelu(x, approximate=True)
def _silu(x):
    return jax.nn.silu(x)
def _sigmoid(x):
    return jax.nn.sigmoid(x)
def _layernorm(x, axis=-1, eps=1e-5):
    m = jnp.mean(x, axis=axis, keepdims=True)
    v = jnp.var(x, axis=axis, keepdims=True)
    return (x - m) / jnp.sqrt(v + eps)
def _scatter_add(tgt, idx, src, axis=0):
    return tgt.at[idx].add(src)
def _segment_sum(src, seg, n):
    return jax.ops.segment_sum(src, seg, n)
class _Rng:
    def __init__(self, key):
        self._k = key
    def _next(self):
        self._k, sub = jax.random.split(self._k)
        return sub
    def normal(self, shape):
        return jax.random.normal(self._next(), shape, dtype=jnp.bfloat16)
    def randint(self, lo, hi, shape):
        return jax.random.randint(self._next(), shape, lo, hi, dtype=jnp.int32)
    def uniform(self, shape, lo=0.0, hi=1.0):
        return jax.random.uniform(self._next(), shape, jnp.bfloat16, lo, hi)
    def permutation(self, n):
        return jax.random.permutation(self._next(), n)


kernel_name = 'interleave_layers__sliding_local_dilated__mixer_s_mlp__prompt'

def setup_inputs():
    _rng = _Rng(jax.random.key(int.from_bytes(__import__("os").urandom(4), "little")))
    _w = (lambda a: (lambda t: t.astype(jnp.bfloat16) if jnp.issubdtype(t.dtype, jnp.floating) else t)(jnp.asarray(a)))
    def _A_setup():
        B, S, D = 1, 2048, 448
        return {
            "x": _w((lambda *s: _rng.normal(s) * 0.05)(B, S, D)),
            "wqkv": _w((lambda *s: _rng.normal(s) * 0.05)(D, 3 * D)),
            "wo": _w((lambda *s: _rng.normal(s) * 0.05)(D, D)),
        }
    _A_in = _A_setup()

    def _B_setup():
        B, S, D, F = 1, 2048, 448, 1792
        return {
            "x":  _w((lambda *s: _rng.normal(s) * 0.05)(B, S, D)),
            "w1": _w((lambda *s: _rng.normal(s) * 0.8)(D, D) * (D ** -0.5)),
            "w2": _w((lambda *s: _rng.normal(s) * 0.8)(D, D) * (D ** -0.5)),
            "w3": _w((lambda *s: _rng.normal(s) * 0.8)(D, F) * (D ** -0.5)),
            "w4": _w((lambda *s: _rng.normal(s) * 0.8)(F, D) * (F ** -0.5)),
        }
    _B_in = _B_setup()

    return {
        "A_x": _A_in["x"],
        "A_wqkv": _A_in["wqkv"],
        "A_wo": _A_in["wo"],
        "B_x": _B_in["x"],
        "B_w1": _B_in["w1"],
        "B_w2": _B_in["w2"],
        "B_w3": _B_in["w3"],
        "B_w4": _B_in["w4"],
    }

def reference(A_x, A_wqkv, A_wo, B_x, B_w1, B_w2, B_w3, B_w4):
    def _A_ref(x, wqkv, wo):
        B, S, D = x.shape
        H = 16; Dh = D // H
        W, dil = 8, 2
        qkv = (lambda x, *d: x.transpose(*d))((x @ wqkv).reshape(B, S, 3, H, Dh), 2, 0, 3, 1, 4)
        q, k, v = qkv[0], qkv[1], qkv[2]
        scale = Dh ** -0.5
        pos = jnp.arange(S)
        off = jnp.arange(W) * dil
        idx = pos[:, None] - off[None, :]
        mask = idx >= 0
        idx_c = jnp.where(mask, idx, 0).reshape(-1)
        kg = k[:, :, idx_c, :].reshape(B, H, S, W, Dh)
        vg = v[:, :, idx_c, :].reshape(B, H, S, W, Dh)
        logits = jnp.einsum("bhsd,bhswd->bhsw", q, kg) * scale
        logits = jnp.where(mask[None, None, :, :], logits, -1e9)
        attn = _softmax(logits, axis=-1)
        o = jnp.einsum("bhsw,bhswd->bhsd", attn, vg)
        return (lambda x, *d: x.transpose(*d))(o, 0, 2, 1, 3).reshape(B, S, D) @ wo

    def _B_ref(x, w1, w2, w3, w4):
        B, S, D = x.shape
        h = _gelu(_layernorm(x, axis=-1) @ w1)
        c = D // 4
        g0 = jnp.pad(h[:, :, 0*c:1*c], ((0, 0), (1, 0), (0, 0)))[:, :S, :]
        g1 = jnp.pad(h[:, :, 1*c:2*c], ((0, 0), (0, 1), (0, 0)))[:, 1:, :]
        g2 = jnp.pad(h[:, :, 2*c:3*c], ((0, 0), (2, 0), (0, 0)))[:, :S, :]
        g3 = jnp.pad(h[:, :, 3*c:   ], ((0, 0), (0, 2), (0, 0)))[:, 2:, :]
        hs = jnp.concatenate([g0, g1, g2, g3], axis=-1) @ w2
        x1 = x + hs
        h2 = _gelu(_layernorm(x1, axis=-1) @ w3) @ w4
        return x1 + h2

    x = A_x
    x = x + _A_ref(_layernorm(x, axis=-1), A_wqkv, A_wo)
    x = x + _B_ref(_layernorm(x, axis=-1), B_w1, B_w2, B_w3, B_w4)
    x = x + _A_ref(_layernorm(x, axis=-1), A_wqkv, A_wo)
    x = x + _B_ref(_layernorm(x, axis=-1), B_w1, B_w2, B_w3, B_w4)
    return x
```

```python
import functools

import jax
import jax.experimental.pallas as pl
import jax.experimental.pallas.tpu as pltpu
import jax.numpy as jnp
import numpy as np
from jax import lax

S, D, F = 2048, 448, 1792
H, DH = 16, 28
W, DIL = 8, 2
GIANT = DIL * W // 2
LAYERS = 2
EPS = 1e-5
NT = S // 128
NG = NT // 2
CHUNK = 32
F32, BF16, I32 = jnp.float32, jnp.bfloat16, jnp.int32
GELU_C0 = float(np.sqrt(2.0 / np.pi))
GELU_C1 = GELU_C0 * 0.044715

SHAPES = dict(qkv=(3 * D, D), wo=(D, D), w1=(D, D), w2=(D, D), w3=(F, D), w4=(D, F))
STAGE_ROW = dict(qkv=0, wo=3 * D // 2, w1=4 * D // 2, w2=5 * D // 2, w3=6 * D // 2, w4=0)
SLOTS = dict(qkv=3, wo=3, w1=3, w2=3, w3=2, w4=4)
EPILOGUE_OPS = dict(qkv=2, wo=8, w1=12, w2=10, w3=18.4, w4=8)

MIN_SHARE, MAX_SHARE, MARGIN, SLACK, HORIZON, XLU_SHARE = 0.4, 0.72, 1.4, 1500, 14000, 0.75
RESULT_LAG, VECTOR_LAG, EPILOGUE_LAG, MATMUL_LAG = 240, 120, 20, 40
RELEASE_DELAY, ANCHOR_DELAY, EPILOGUE_ANCHOR_DELAY = 300, 50, 200
DMA_DUE = (0, 0, 1700, 6700, 13500)
DMA_AFTER = (-1, -1, 0, 2, 3)


def _gelu2(x):
    t = lax.tanh(lax.mul(x, lax.add(lax.mul(lax.mul(x, x), np.float32(GELU_C1)), np.float32(GELU_C0))))
    return lax.add(lax.mul(x, t), x)


def _pack(lo, hi):
    return pltpu.bitcast(pltpu.pack_elementwise([lo, hi], packed_dtype=BF16), I32)


def _unpack(w, i):
    return pltpu.unpack_elementwise(w, index=i, packed_dtype=BF16, unpacked_dtype=F32)


def _as_bf16(x):
    return pltpu.bitcast(x, BF16)


def _lhs_terms(grid):
    (a11, a12), (a21, a22) = grid
    return [lax.add(a11, a22), lax.add(a21, a22), a11, a22, lax.add(a11, a12), lax.sub(a21, a11), lax.sub(a12, a22)]


def _rhs_terms(grid):
    (b11, b12), (b21, b22) = grid
    return [lax.add(b11, b22), b11, lax.sub(b12, b22), lax.sub(b21, b11), b22, lax.add(b11, b12), lax.add(b21, b22)]


def _block_product(product, out):
    m1 = product(0)
    yield m1
    m2 = product(1)
    yield m2
    c22 = lax.sub(m1, m2)
    m4 = product(3)
    yield m4
    c21, c11 = lax.add(m2, m4), lax.add(m1, m4)
    m3 = product(2)
    yield m3
    c22 = lax.add(c22, m3)
    m5 = product(4)
    yield m5
    c12, c11 = lax.add(m3, m5), lax.sub(c11, m5)
    m6 = product(5)
    yield m6
    c22 = lax.add(c22, m6)
    m7 = product(6)
    yield m7
    out.extend([[lax.add(c11, m7), c12], [c21, c22]])


class _Task:
    def __init__(self, emit, deps, work=0, mxu=0, anchored=True):
        self.emit, self.deps, self.work, self.mxu, self.anchored = emit, list(deps), work, mxu, anchored
        self.deadline = self.done_at = self.steps = self.epilogue = None
        self.is_epilogue, self.uses_xlu = False, True
        self.spent = self.earliest = 0


def _once(f, valu=0, xlu=0):
    def emit():
        f()
        yield valu, xlu
    return emit


def _emit_program(matmuls, anchors, released):
    vector = []

    def visit(task, deadline):
        for d in task.deps:
            if d.mxu == 0 and d.deadline is None:
                d.deadline = deadline
                visit(d, deadline)
                vector.append(d)

    start, free = [0.0], [0.0]
    for i, task in enumerate(matmuls):
        visit(task, i)
        start.append(start[-1] + task.mxu)
        free.append(free[-1] + 4 * task.mxu - task.work - task.epilogue.work)
    pending = [f for f in vector if not f.is_epilogue]
    epilogues, delayed, issued = [], [], []
    clock = valu_credit = xlu_credit = 0

    def step(f):
        if f.steps is None:
            assert all(d.done_at is not None for d in f.deps)
            f.steps = f.emit()
        cost = next(f.steps, None)
        if cost is None:
            f.done_at = clock
        elif not f.mxu:
            f.spent += cost[0]
            if f.anchored:
                due = clock + (EPILOGUE_ANCHOR_DELAY if f.is_epilogue else ANCHOR_DELAY)
                delayed.extend((due, value) for value in cost[2:])
        return cost

    def finish(f):
        if f.done_at is None:
            for d in f.deps:
                finish(d)
            while step(f) is not None:
                pass

    for i, task in enumerate(matmuls):
        if not all(d.done_at is not None and d.done_at + MATMUL_LAG <= clock for d in task.deps):
            for d in task.deps:
                finish(d)
            epilogues = [f for f in epilogues if f.done_at is None]
            pending = [f for f in pending if f.done_at is None]
        need = due = 0.0
        for f in pending:
            if start[f.deadline] - start[i] > HORIZON:
                break
            due += max(f.work - f.spent, 0)
            need = max(need, due / max(free[f.deadline] - free[i] - SLACK, 1.0))
        share = min(max(MARGIN * need, MIN_SHARE), MAX_SHARE)
        cycles = task.mxu / 7
        while (result := step(task)) is not None:
            issued.append((clock + RELEASE_DELAY, result))
            clock += cycles
            valu_credit = min(valu_credit, 0.0) + (share * (free[i + 1] - free[i]) + task.epilogue.work) * cycles / task.mxu
            xlu_credit = min(xlu_credit, 0.0) + XLU_SHARE * cycles
            while issued and issued[0][0] <= clock:
                released[:] = [issued.pop(0)[1]]
            anchors.extend(value for when, value in delayed if when <= clock)
            delayed[:] = [(when, value) for when, value in delayed if when > clock]
            for f in epilogues[:1]:
                quota = 4 * cycles
                while f.deps[0].done_at + EPILOGUE_LAG <= clock and quota > 0 and (cost := step(f)) is not None:
                    valu_credit -= cost[0]
                    quota -= cost[0]
            epilogues = [f for f in epilogues if f.done_at is None]
            for f in pending:
                if valu_credit <= 0 or start[f.deadline] - start[i + 1] > HORIZON:
                    break
                if f.earliest > clock or f.steps is None and not all(
                        d.done_at is not None and d.done_at + (RESULT_LAG if d.is_epilogue else VECTOR_LAG) <= clock
                        for d in f.deps):
                    continue
                while valu_credit > 0 and (xlu_credit > 0 or not f.uses_xlu) and (cost := step(f)) is not None:
                    f.uses_xlu = cost[1] > 0
                    valu_credit -= cost[0]
                    xlu_credit -= cost[1]
            pending = [f for f in pending if f.done_at is None]
        epilogues.append(task.epilogue)
    for f in epilogues:
        finish(f)
    assert not pending


def _matmul_order():
    order = [("qkv", g, part, part + 1, 3) for part in range(3) for g in range(3)]
    order += [("qkv", 3), ("qkv", 4), ("wo", 0), ("qkv", 5), ("w1", 0), ("wo", 1), ("qkv", 6), ("w1", 1),
              ("qkv", 7, 0, 2, 7), ("w2", 0), ("qkv", 7, 2, 5, 7)]
    ramp = 3
    for s in range(ramp + 1):
        order += [("w3", s), ("qkv", s + 7, 5, 7, 7), ("w4", s, 0, 4, 7), ("wo", s + 2)]
        if s < ramp:
            order += [("w4", s, 4, 7, 7), ("w1", s + 2), ("qkv", s + 8, 0, 2, 7), ("w2", s + 1), ("qkv", s + 8, 2, 5, 7)]
    order += [("w4", ramp, 4, 6, 7), ("w1", ramp + 2), ("w4", ramp, 6, 7, 7), ("w2", ramp + 1), ("wo", ramp + 3)]
    last = LAYERS * NG - 1
    for s in range(ramp + 1, last + 1):
        order += [("w3", s), ("w1", s + 2)]
        if s >= last - 1:
            order += [("w4", s - 1, 5, 7, 7)]
        order += [("w4", s, 0, 3, 7), ("w2", s + 1), ("w4", s, 3, 5 if last - 2 <= s < last else 7, 7), ("qkv", s + 7),
                  ("wo", s + 3)]
    return order


def _first_output(name, i, r):
    if name == "qkv":
        part, rest = divmod(r, D // 2)
        return (1, 0, 2)[part] * D + i * (D // 2) + rest
    return i * (SHAPES[name][0] // 2) + r


def _kernel(x_hbm, wqkv_hbm, wo_hbm, w1_hbm, w2_hbm, w3_hbm, w4_hbm, out_hbm,
            xin, obuf, xres, ybuf, hbuf, q_s, k_s, v_s, near_s, far_s, logit_s, prob_s, stage_s, wo_s, w4_s, *rest):
    names = list(SHAPES)
    raw, lhs, rhs = (dict(zip(names, rest[i:i + 6])) for i in (0, 6, 12))
    in_sem, out_sem = rest[18:]

    cols = lambda src, dst, a, b: (src.at[:, pl.ds(a, b - a)], dst.at[:, pl.ds(a, b - a)])
    out_copy = [pltpu.make_async_copy(*cols(obuf, out_hbm, g * 256, (g + 1) * 256), out_sem.at[g]) for g in range(NG)]
    batches = [[cols(x_hbm, xin, 0, 512)],
               [cols(wqkv_hbm, raw["qkv"], 384, 896), cols(x_hbm, xin, 512, 768)],
               [cols(wqkv_hbm, raw["qkv"], 0, 384), cols(wqkv_hbm, raw["qkv"], 896, 3 * D), cols(x_hbm, xin, 768, 1024)],
               [cols(x_hbm, xin, 1024, S), (wo_hbm, raw["wo"]), (w1_hbm, raw["w1"]), (w2_hbm, raw["w2"])],
               [(w3_hbm, raw["w3"]), (w4_hbm, raw["w4"])]]
    copies, count = [], 0
    for batch in batches:
        copies.append([pltpu.make_async_copy(src, dst, in_sem.at[count + i]) for i, (src, dst) in enumerate(batch)])
        count += len(batch)

    def start_after(i):
        for batch, after in zip(copies, DMA_AFTER):
            if after == i:
                for c in batch:
                    c.start()

    def arrive(i):
        for c in copies[i]:
            c.wait()
        start_after(i)

    start_after(-1)
    arrived = []
    for i in range(len(copies)):
        arrived.append(_Task(_once(functools.partial(arrive, i)), arrived[-1:]))
        arrived[-1].earliest = DMA_DUE[i]
    weight_arrived = dict(qkv=arrived[2], wo=arrived[3], w1=arrived[3], w2=arrived[3], w3=arrived[4], w4=arrived[4])

    lane = lax.broadcasted_iota(I32, (8, 128), 1)
    from_lane = functools.cache(lambda n: lane >= n)
    zeros = lambda: jnp.zeros((8, 128), F32)

    def shift_right(prev, cur, n):
        return pltpu.roll(lax.select(from_lane(128 - n), prev, cur), n, axis=1)

    def shift_left(cur, nxt, n):
        return pltpu.roll(lax.select(from_lane(n), cur, nxt), 128 - n, axis=1)

    anchors, released = [], []

    @functools.cache
    def never():
        w = pltpu.bitcast(xin[0:16, 0:128], I32)
        return ((w * w) & 2) != 0

    def gate(x):
        if not released:
            return x
        return lax.select(never(), released[0] if x.dtype == F32 else pltpu.bitcast(released[0], I32), x)

    def tie(w):
        if not anchors:
            return w
        head = w[0:8, 0:128]
        tree = [a if a.dtype == I32 else pltpu.bitcast(a, I32) for a in anchors]
        while len(tree) > 1:
            tree = [lax.bitwise_or(a, b) for a, b in zip(tree[::2], tree[1::2])] + tree[len(tree) // 2 * 2:]
        head = lax.select(never(), tree[0], head)
        anchors.clear()
        return jnp.concatenate([jnp.concatenate([head, w[0:8, 128:]], axis=1), w[8:]], axis=0)

    def prepare_weight(name):
        m, k = SHAPES[name]
        panels = [(c, min(128, k // 2 - c)) for c in range(0, k // 2, 128)]
        row0 = STAGE_ROW[name]
        if name == "w4":
            def copy_panel(c):
                for r in range(0, m, 64):
                    w4_s[c // 128, r // 2:r // 2 + 32] = pltpu.bitcast(raw[name][r:r + 64, c:c + 128], I32)
                    yield 4, 0
            staged = [_Task(functools.partial(copy_panel, c), [weight_arrived[name]], work=28) for c in range(0, k, 128)]
            words = lambda j, p, rows: w4_s[j * len(panels) + p, rows]
        else:
            ready = [weight_arrived[name]]
            if name == "wo":
                def widen(c):
                    cw = min(128, D - c)
                    for r in range(0, D, 32):
                        wo_s[c // 128, r:r + 32, 0:cw] = raw[name][r:r + 32, c:c + cw].astype(F32)
                        yield 8, 0
                ready = [_Task(functools.partial(widen, c), ready, work=112) for c in range(0, D, 128)]

            def transpose(j, p, c):
                k0, kw = panels[p]
                cw = min(128, m - c)
                r0 = j * (k // 2) + k0
                if name == "wo":
                    heads = lambda d, h: wo_s[c // 128, pl.ds(h * DH + d, 8, stride=DH), 0:cw]
                    src = [_pack(heads(d, 0), heads(d, 8)) for d in range(r0 // H, (r0 + kw) // H)]
                else:
                    src = [pltpu.bitcast(raw[name][r:r + 16, c:c + cw], I32) for r in range(r0, r0 + kw, 16)]
                if cw == 128:
                    src[0] = gate(src[0])
                stage_s[j * len(panels) + p, row0 + c // 2:row0 + (c + cw) // 2, 0:kw] = pltpu.bitcast(
                    _as_bf16(jnp.concatenate(src, axis=0)).T, I32)

            staged = {c: [_Task(_once(functools.partial(transpose, j, p, c), 40, 28),
                                [arrived[1]] if name == "qkv" and 384 <= c < 896 else ready, work=40)
                          for j in range(2) for p in range(len(panels))] for c in range(0, m, 128)}
            words = lambda j, p, rows: stage_s[j * len(panels) + p, rows, 0:panels[p][1]]
        halved = name in ("w2", "w4")
        cost = 1.1 * (8 * halved + 24.5)

        def combine(r):
            def terms(grid, halves):
                grid = [[_unpack(v, e) for v in row] for row, e in zip(grid, halves)]
                if halved:
                    grid = [[lax.mul(v, np.float32(0.5)) for v in row] for row in grid]
                return _lhs_terms(grid)

            first = [_first_output(name, i, r) for i in range(2)]
            for p, (c, kw) in enumerate(panels):
                load = lambda rows: [[words(j, p, rows(row)) for j in range(2)] for row in first]
                if name == "qkv":
                    rows = lambda h: lambda row: pl.ds(row0 + (row // D * D + h * DH + row % D // H) // 2, 8, stride=DH)
                    todo = [(load(rows(0)), load(rows(1)), [row % D // H % 2 for row in first], r)]
                else:
                    a, b = (load(lambda row: pl.ds(row0 + row // 2 + s, 8, stride=2)) for s in range(2))
                    todo = [(a, b, [e, e], r + 16 * e) for e in range(2)]
                for a, b, halves, dst in todo:
                    packed = [_pack(lo, hi) for lo, hi in zip(terms(a, halves), terms(b, halves))]
                    for i, word in enumerate(packed):
                        lhs[name][i, dst // 2:dst // 2 + 8, c:c + kw] = word
                    yield (cost, 0, *packed) if kw == 128 else (cost - 7, 0)

        def inputs_of(r, size):
            if name == "w4":
                return staged
            spans = [(_first_output(name, i, r), _first_output(name, i, r) + size) for i in range(2)]
            if name == "qkv":
                spans = [(a // D * D, a // D * D + D) for a, _ in spans]
            return [t for c, ts in staged.items() if any(c < b and a < c + 128 for a, b in spans) for t in ts]

        size = 16 if name == "qkv" else CHUNK
        return {r0: [_Task(functools.partial(combine, r), inputs_of(r, size), work=len(panels) * size // 16 * cost)
                     for r in range(r0, r0 + CHUNK, size)] for r0 in range(0, m // 2, CHUNK)}

    weight_ready = {name: prepare_weight(name) for name in names}

    overwrites = []
    readers = {name: {} for name in names}

    def store_rhs(name, g, r, grid):
        lo = _rhs_terms([[v[0] for v in row] for row in grid])
        hi = _rhs_terms([[v[1] for v in row] for row in grid])
        for i, (a, b) in enumerate(zip(lo, hi)):
            word = _pack(a, b)
            rhs[name][g % SLOTS[name], i, r // 2:r // 2 + 8, :] = word
            yield (3.5, 0, word) if name != "w4" else (2.5, 0)

    def prepare_rhs(name, groups, produce, deps, valu, xlu=0):
        half = SHAPES[name][1] // 2
        tasks = {}
        for g, tiles in groups:
            def emit(r, g=g, tiles=tiles):
                grid = []
                for i in range(2):
                    grid.append([produce(i * half + r, t) for t in tiles])
                    yield 2 * valu, 2 * xlu
                yield from store_rhs(name, g, r, grid)
            tasks[g] = [_Task(functools.partial(emit, r), deps(tiles, [r, half + r]), work=4 * valu + 24.5)
                        for r in range(0, half, 16)]
            overwrites.extend((t, name, g) for t in tasks[g])
        return tasks

    def matmul(name, groups, rhs_ready, consume):
        m, k = SHAPES[name]
        passes = -(-(k // 2) // 128)
        if name == "qkv":
            pieces = [(0, slice(0, 8), slice(8, 16)), (16, slice(16, 24), slice(24, 32))]
        else:
            pieces = [(0, slice(0, 8), slice(16, 24)), (16, slice(8, 16), slice(24, 32))]
        tasks = []
        for g, tiles in groups:
            tasks.append([])
            for r in range(0, m // 2, CHUNK):
                blocks = []

                def emit(r=r, g=g, blocks=blocks):
                    product = lambda i: lax.dot_general(
                        _as_bf16(tie(lhs[name][i, r // 2:(r + CHUNK) // 2, :])), _as_bf16(rhs[name][g % SLOTS[name], i]),
                        (((1,), (0,)), ((), ())), preferred_element_type=F32)
                    for value in _block_product(product, blocks):
                        yield value[0:8]

                def epilogue(r=r, g=g, tiles=tiles, blocks=blocks):
                    for o, lo, hi in pieces:
                        yield from consume(g, tiles, [_first_output(name, i, r + o) for i in range(2)],
                                           [[(v[lo], v[hi]) for v in row] for row in blocks])

                task = _Task(emit, rhs_ready[g] + weight_ready[name][r], mxu=7 * passes * CHUNK / 4,
                             work=7 * (passes - 1 + 8 / 7) * CHUNK / 8)
                task.epilogue = _Task(epilogue, [task], work=EPILOGUE_OPS[name] * 4 * CHUNK / 16,
                                      anchored=name in ("wo", "w2", "w4"))
                task.epilogue.is_epilogue = True
                task.rows = [_first_output(name, i, u) for i in range(2) for u in range(r, r + CHUNK, 16)]
                task.tiles = tiles
                tasks[-1].append(task)
                readers[name].setdefault(g, []).append(task)
                if name == "w3":
                    overwrites.append((task, "w4", g))
        return tasks

    def writers(tasks, t, r0=0, r1=S):
        return [k.epilogue for ks in tasks for k in ks if t in k.tiles and any(a < r1 and r0 < a + 16 for a in k.rows)]

    def each_pair(f, valu):
        def consume(g, tiles, rows, blocks):
            for r, row in zip(rows, blocks):
                for t, (lo, hi) in zip(tiles, row):
                    yield valu, 0, *f(r, t, lo, hi)
        return consume

    def put(ref, t, r, lo, hi):
        ref[t, r:r + 8] = lo
        ref[t, r + 8:r + 16] = hi

    class LayerNorm:
        def __init__(self):
            self.sums, self.moments, self.count = {}, {}, {}

        def add(self, t, lo, hi):
            s1, s2 = lax.add(lo, hi), lax.add(lax.mul(lo, lo), lax.mul(hi, hi))
            if t in self.sums:
                s1, s2 = lax.add(self.sums[t][0], s1), lax.add(self.sums[t][1], s2)
            self.sums[t] = s1, s2
            self.count[t] = self.count.get(t, 0) + 1
            return (s1, s2)[self.count[t] % 2],

        def finish(self, t, deps):
            def emit():
                mean, sq = (jnp.broadcast_to(jnp.sum(v, axis=0, keepdims=True), (8, 128)) * (1.0 / D) for v in self.sums[t])
                rstd = lax.rsqrt(jnp.maximum(sq - mean * mean, 0.0) + EPS)
                self.moments[t] = mean, rstd
                yield 30, 0, rstd
            return _Task(emit, deps, work=30)

        def apply(self, ref):
            def rows(r, t):
                mean, rstd = gate(self.moments[t][0]), self.moments[t][1]
                return [lax.mul(lax.sub(ref[t, u:u + 8], mean), rstd) for u in (r, r + 8)]
            return rows

    def layer(index, previous, ln1):
        groups = [(index * NG + g, [2 * g, 2 * g + 1]) for g in range(NG)]
        mm = {}
        if index == 0:
            def widen(t):
                for r in range(0, D, 16):
                    word = gate(pltpu.bitcast(xin[r:r + 16, t * 128:(t + 1) * 128], I32))
                    lo, hi = _unpack(word, 0), _unpack(word, 1)
                    put(xres, t, r, lo, hi)
                    yield 9, 0, *ln1.add(t, lo, hi)
            source = [[_Task(functools.partial(widen, t), [arrived[0 if t < 4 else min(t // 2 - 1, 3)]], work=252)]
                      for t in range(NT)]
        else:
            source = [writers(previous, t) for t in range(NT)]
        norm1 = [ln1.finish(t, source[t]) for t in range(NT)]

        def put_qkv(row, t, lo, hi):
            put((q_s, k_s, v_s)[row // D], t, row % D, lo, hi)
            return lo, hi

        mm["qkv"] = matmul("qkv", groups, prepare_rhs("qkv", groups, ln1.apply(xres),
                                                      lambda tiles, rows: [norm1[t] for t in tiles], 5),
                           each_pair(put_qkv, 2))

        def logits(t, e):
            acc = [None] * W
            for d in range(DH):
                rows = slice(d * H + 8 * e, d * H + 8 * e + 8)
                kc, kp = gate(k_s[t, rows]), k_s[t - 1, rows] if t else zeros()
                q0 = gate(q_s[t, rows])
                q1 = shift_left(q0, q_s[t + 1, rows] if t + 1 < NT else zeros(), GIANT)
                for j in range(W // 2):
                    kj = shift_right(kp, kc, DIL * j) if j else kc
                    for w, q in ((j, q0), (W // 2 + j, q1)):
                        acc[w] = lax.add(acc[w], lax.mul(q, kj)) if d else lax.mul(q, kj)
                yield 23, 10.7, acc[d * 3 % W]
            for w in range(W):
                logit_s[t, w, 8 * e:8 * e + 8] = acc[w] * (DH ** -0.5)

        def softmax(t, e):
            rows = slice(8 * e, 8 * e + 8)
            ls = []
            for w in range(W):
                logit = logit_s[t, w, rows]
                if w >= W // 2:
                    logit = shift_right(logit_s[t - 1, w, rows] if t else zeros(), logit, GIANT)
                ls.append(jnp.where(lane >= DIL * w, logit, -1e9) if t == 0 and w else logit)
            top = functools.reduce(jnp.maximum, ls)
            es = [jnp.exp(logit - top) for logit in ls]
            inv = 1.0 / functools.reduce(lambda a, b: a + b, es)
            for w in range(W):
                prob_s[t, w, rows] = es[w] * inv
            yield 65, 11, inv

        def move_probs(t, e):
            rows = slice(8 * e, 8 * e + 8)
            for w in range(W // 2, W):
                moved = shift_left(prob_s[t, w, rows], prob_s[t + 1, w, rows] if t + 1 < NT else zeros(), GIANT)
                prob_s[t, W // 2 + w, rows] = moved
                yield 2, 2.7, moved

        def sequence_start():
            masked = []
            for rows in (slice(0, 8), slice(8, 16)):
                p = [prob_s[0, w, rows] for w in range(W // 2, W)]
                masked.append(pltpu.roll((p[0] + p[1]) + (p[2] + p[3]), 128 - GIANT, axis=1))
            for r in range(0, D, 8):
                first = lax.select(from_lane(1), zeros(), gate(v_s[0, r:r + 8]))
                first = jnp.broadcast_to(jnp.sum(first, axis=1, keepdims=True), (8, 128))
                far_s[NT, r:r + 8] = first
                carried = lax.mul(masked[r % H // 8], first)
                far_s[NT + 1, r:r + 8] = carried
                yield 4, 4, carried

        def mix(t, d):
            for e in range(2):
                rows, heads = slice(d * H + 8 * e, d * H + 8 * e + 8), slice(8 * e, 8 * e + 8)
                vc = gate(v_s[t, rows])
                vp = v_s[t - 1, rows] if t else far_s[NT, rows]
                near = far = None
                for j in range(W // 2):
                    vj = shift_right(vp, vc, DIL * j) if j else vc
                    a, b = lax.mul(prob_s[t, j, heads], vj), lax.mul(prob_s[t, W + j, heads], vj)
                    near, far = (lax.add(near, a), lax.add(far, b)) if j else (a, b)
                far_s[t, rows] = far
                near_s[t, rows] = near
                yield 20, 8, near, far

        def attended(r, t):
            before = far_s[t - 1 if t else NT + 1, r:r + 8]
            return lax.add(near_s[t, r:r + 8], shift_right(before, gate(far_s[t, r:r + 8]), GIANT))

        back = lambda t: [u for u in (t - 1, t) if u >= 0]
        ahead = lambda t: [u for u in (t, t + 1) if u < NT]
        halves = [(t, e) for t in range(NT) for e in range(2)]
        scored = {(t, e): _Task(functools.partial(logits, t, e),
                                [k for u in back(t) for k in writers(mm["qkv"], u, D, 2 * D)]
                                + [k for u in ahead(t) for k in writers(mm["qkv"], u, 0, D)], work=644) for t, e in halves}
        normed = {(t, e): _Task(functools.partial(softmax, t, e), [scored[u, e] for u in back(t)], work=65) for t, e in halves}
        moved = {(t, e): _Task(functools.partial(move_probs, t, e), [normed[u, e] for u in ahead(t)], work=8) for t, e in halves}
        start = _Task(sequence_start, [normed[0, 0], normed[0, 1]] + writers(mm["qkv"], 0, 2 * D), work=224)
        mixed = {(t, d): _Task(functools.partial(mix, t, d), [moved[t, 0], moved[t, 1]]
                               + [k for u in back(t) for k in writers(mm["qkv"], u, 2 * D + d * H, 2 * D + (d + 1) * H)]
                               + ([] if t else [start]), work=40) for t in range(NT) for d in range(DH)}
        ln2, ln3, ln4, ln_next = LayerNorm(), LayerNorm(), LayerNorm(), LayerNorm()

        def put_attention(r, t, lo, hi):
            lo, hi = lax.add(xres[t, r:r + 8], lo), lax.add(xres[t, r + 8:r + 16], hi)
            put(xres, t, r, lo, hi)
            return ln2.add(t, lo, hi)

        mm["wo"] = matmul("wo", groups, prepare_rhs(
            "wo", groups, lambda r, t: (attended(r, t), attended(r + 8, t)),
            lambda tiles, rows: [mixed[u, r // H] for r in rows for t in tiles for u in back(t)], 6, 5.4),
            each_pair(put_attention, 8))

        def block_input(t):
            for r in range(0, D, 16):
                lo, hi = ln2.apply(xres)(r, t)
                put(ybuf, t, r, lo, hi)
                yield 10, 0, *ln3.add(t, lo, hi)

        norm3 = [ln3.finish(t, [_Task(functools.partial(block_input, t), [ln2.finish(t, writers(mm["wo"], t))], work=280)])
                 for t in range(NT)]

        def put_hidden(r, t, lo, hi):
            lo, hi = _gelu2(lo), _gelu2(hi)
            put(hbuf, t, r, lo, hi)
            return lo, hi

        mm["w1"] = matmul("w1", groups, prepare_rhs("w1", groups, ln3.apply(ybuf),
                                                    lambda tiles, rows: [norm3[t] for t in tiles], 5),
                          each_pair(put_hidden, 12))
        shift_of = lambda r: (1, -1, 2, -2)[r // (D // 4)]
        neighbour = lambda r, t: t - 1 if shift_of(r) > 0 else t + 1

        def shifted(r, t):
            n, u = shift_of(r), neighbour(r, t)
            cur = gate(hbuf[t, r:r + 8])
            other = hbuf[u, r:r + 8] if 0 <= u < NT else zeros()
            return shift_right(other, cur, n) if n > 0 else shift_left(cur, other, -n)

        def put_mixed(r, t, lo, hi):
            lo, hi = lax.add(ybuf[t, r:r + 8], lo), lax.add(ybuf[t, r + 8:r + 16], hi)
            put(ybuf, t, r, lo, hi)
            put(xres, t, r, lax.add(xres[t, r:r + 8], lo), lax.add(xres[t, r + 8:r + 16], hi))
            return ln4.add(t, lo, hi)

        mm["w2"] = matmul("w2", groups, prepare_rhs(
            "w2", groups, lambda r, t: (shifted(r, t), shifted(r + 8, t)),
            lambda tiles, rows: [k for r in rows for t in tiles for u in (t, neighbour(r, t))
                                 for k in writers(mm["w1"], u, r, r + 16)], 4, 11), each_pair(put_mixed, 10))
        norm4 = [ln4.finish(t, writers(mm["w2"], t)) for t in range(NT)]

        def put_expanded(g, tiles, rows, blocks):
            grid = []
            for row in blocks:
                grid.append([])
                for lo, hi in row:
                    grid[-1].append((_gelu2(lo), _gelu2(hi)))
                    yield 14, 0
            yield from store_rhs("w4", g, rows[0], grid)

        mm["w3"] = matmul("w3", groups, prepare_rhs("w3", groups, ln4.apply(ybuf),
                                                    lambda tiles, rows: [norm4[t] for t in tiles], 5), put_expanded)

        def put_result(r, t, lo, hi):
            lo, hi = lax.add(xres[t, r:r + 8], lo), lax.add(xres[t, r + 8:r + 16], hi)
            if index == LAYERS - 1:
                word = _pack(lo, hi)
                obuf[r:r + 16, t * 128:(t + 1) * 128] = _as_bf16(word)
                return word,
            put(xres, t, r, lo, hi)
            return ln_next.add(t, lo, hi)

        mm["w4"] = matmul("w4", groups, {g: [k.epilogue for k in ks] for (g, _), ks in zip(groups, mm["w3"])},
                          each_pair(put_result, 8))
        return mm, ln_next

    layers, norm = [], LayerNorm()
    for index in range(LAYERS):
        mm, norm = layer(index, layers[-1]["w4"] if index else None, norm)
        layers.append(mm)
    for task, name, g in overwrites:
        task.deps += readers[name].get(g - SLOTS[name], [])

    for g, tasks in enumerate(layers[-1]["w4"]):
        left = [len(tasks)]
        for task in tasks:
            def epilogue(inner=task.epilogue.emit, left=left, g=g):
                yield from inner()
                left[0] -= 1
                if not left[0]:
                    out_copy[g].start()
            task.epilogue.emit = epilogue

    sequence = []
    for name, g, *part in _matmul_order():
        first, last, parts = part or (0, 1, 1)
        if g < LAYERS * NG:
            tasks = layers[g // NG][name][g % NG]
            sequence.extend(tasks[len(tasks) * first // parts:len(tasks) * last // parts])
    assert len(sequence) == sum(len(ts) for mm in layers for groups in mm.values() for ts in groups)
    _emit_program(sequence, anchors, released)
    for c in out_copy:
        c.wait()


@jax.jit
def pallas_interleave_layers__sliding_local_dilated__mixer_s_mlp__prompt_kernel(
    A_x: jax.Array,
    A_wqkv: jax.Array,
    A_wo: jax.Array,
    B_x: jax.Array,
    B_w1: jax.Array,
    B_w2: jax.Array,
    B_w3: jax.Array,
    B_w4: jax.Array,
):
    del B_x
    hbm = pl.BlockSpec(memory_space=pl.ANY)
    vmem = pltpu.VMEM
    out = pl.pallas_call(
        _kernel,
        out_shape=jax.ShapeDtypeStruct((D, S), BF16),
        in_specs=[hbm] * 7,
        out_specs=hbm,
        scratch_shapes=[
            vmem((D, S), BF16), vmem((D, S), BF16),
            *[vmem((NT, D, 128), F32) for _ in range(7)], vmem((NT + 2, D, 128), F32),
            vmem((NT, W, H, 128), F32), vmem((NT, W + W // 2, H, 128), F32),
            vmem((4, 5 * D + 8, 128), I32), vmem((4, D + 32, 128), F32), vmem((F // 128, D // 2 + 8, 128), I32),
            vmem((D, 3 * D), BF16), vmem((D, D), BF16), vmem((D, D), BF16), vmem((D, D), BF16),
            vmem((D, F), BF16), vmem((D, F), BF16),
            *[vmem((7, m // 4, k // 2), I32) for m, k in SHAPES.values()],
            *[vmem((SLOTS[name], 7, k // 4, 128), I32) for name, (_, k) in SHAPES.items()],
            pltpu.SemaphoreType.DMA((12,)), pltpu.SemaphoreType.DMA((NG,)),
        ],
        compiler_params=pltpu.CompilerParams(vmem_limit_bytes=120 * 2 ** 20),
        name="fusedk",
    )(A_x.reshape(S, D).T, A_wqkv, A_wo, B_w1, B_w2, B_w3, B_w4.T)
    return out.T.reshape(1, S, D)
```
